```python
import os as _os
_os.environ.setdefault("JAX_PLATFORMS", "cpu")
import jax
import jax.numpy as jnp

def _softmax(x, axis=-1):
    return jax.nn.softmax(x, axis=axis)
def _gelu(x):
    return jax.nn.gelu(x, approximate=True)
def _silu(x):
    return jax.nn.silu(x)
def _sigmoid(x):
    return jax.nn.sigmoid(x)
def _layernorm(x, axis=-1, eps=1e-5):
    m = jnp.mean(x, axis=axis, keepdims=True)
    v = jnp.var(x, axis=axis, keepdims=True)
    return (x - m) / jnp.sqrt(v + eps)
def _scatter_add(tgt, idx, src, axis=0):
    return tgt.at[idx].add(src)
def _segment_sum(src, seg, n):
    return jax.ops.segment_sum(src, seg, n)
class _Rng:
    def __init__(self, key):
        self._k = key
    def _next(self):
        self._k, sub = jax.random.split(self._k)
        return sub
    def normal(self, shape):
        return jax.random.normal(self._next(), shape, dtype=jnp.bfloat16)
    def randint(self, lo, hi, shape):
        return jax.random.randint(self._next(), shape, lo, hi, dtype=jnp.int32)
    def uniform(self, shape, lo=0.0, hi=1.0):
        return jax.random.uniform(self._next(), shape, jnp.bfloat16, lo, hi)
    def permutation(self, n):
        return jax.random.permutation(self._next(), n)


kernel_name = 'standalone__geglu_ffn__prompt'

def setup_inputs():
    _rng = _Rng(jax.random.key(int.from_bytes(__import__("os").urandom(4), "little")))
    _w = (lambda a: (lambda t: t.astype(jnp.bfloat16) if jnp.issubdtype(t.dtype, jnp.floating) else t)(jnp.asarray(a)))
    B, S, D, F = 1, 2048, 576, 4608
    return {
        "x": _w((lambda *s: _rng.normal(s) * 0.05)(B, S, D)),
        "w_gate": _w((lambda *s: _rng.normal(s) * 0.05)(D, F)),
        "w_up": _w((lambda *s: _rng.normal(s) * 0.05)(D, F)),
        "w_down": _w((lambda *s: _rng.normal(s) * 0.05)(F, D)),
    }

def reference(x, w_gate, w_up, w_down):
    return (_gelu(x @ w_gate) * (x @ w_up)) @ w_down
```

```python
import jax
import jax.numpy as jnp
from jax import lax
import jax.experimental.pallas as pl
import jax.experimental.pallas.tpu as pltpu

_NT = (((1,), (1,)), ((), ()))
_BF = jnp.bfloat16
_F32 = jnp.float32

_D, _M, _F = 576, 2048, 4608
_TM = 512
_HM = _TM // 2
_C0 = 256
_C = 512
_TFL = 512
_NL = (_F - _C) // _TFL
_G1 = _C + _TFL
_NSUB = _M // _TM
_TAIL = 128


def _gelu(g):
    c = 0.7978845608028654
    return 0.5 * g * (1.0 + jnp.tanh(c * (g + 0.044715 * (g * g * g))))


def _kernel(xT_hbm, wg_hbm, wu_hbm, wdT_hbm, oT_hbm,
            xT_v, xp, xs, wg_v, wu_v, wd_v, acc, o_v, sems):
    W = [(wg_hbm, wg_v), (wu_hbm, wu_v), (wdT_hbm, wd_v)]

    def cx(a, b, s):
        return pltpu.make_async_copy(xT_hbm.at[:, a:b], xT_v.at[:, a:b], sems.at[s])

    def cw(k, a, b, s):
        h, v = W[k]
        return pltpu.make_async_copy(h.at[:, a:b], v.at[:, a:b], sems.at[s])

    def co(a, b):
        return pltpu.make_async_copy(o_v.at[:, a:b], oT_hbm.at[:, a:b], sems.at[7])

    groups = [
        [cx(0, 128, 0), cx(256, 384, 0)],
        [cw(0, 0, _C0, 1), cw(1, 0, _C0, 1)],
        [cx(128, 256, 2), cx(384, 512, 2), cw(2, 0, _C0, 2)],
        [cx(512, 1024, 3)],
        [cx(1024, _M, 4)] + [cw(k, _C0, _C, 4) for k in range(3)],
        [cw(k, _C, _G1, 5) for k in range(3)],
        [cw(k, _G1, _F, 6) for k in range(3)],
    ]
    for g in groups:
        for c in g:
            c.start()

    def wait(gi):
        for c in groups[gi]:
            c.wait()

    def prep(t, o, n):
        a = t * _TM + o
        b = a + _HM
        s = t * _HM + o
        A, B = slice(a, a + n), slice(b, b + n)
        a8 = xT_v[448:512, A]
        b8 = xT_v[448:512, B]
        a9 = xT_v[512:576, A]
        b9 = xT_v[512:576, B]
        dA = (a8.astype(_F32) - b8.astype(_F32)).astype(_BF)
        dB = (b9.astype(_F32) - a9.astype(_F32)).astype(_BF)
        xp[A, :] = jnp.concatenate([xT_v[0:448, A], dA], axis=0).T
        xp[B, :] = jnp.concatenate([xT_v[0:448, B], dB], axis=0).T
        xs[s:s + n, :] = jnp.concatenate([b8, a9], axis=0).T

    def proj(w, t, o, n, fs):
        a = t * _TM + o
        b = a + _HM
        s = t * _HM + o
        gA = jnp.dot(xp[a:a + n, :], w[0:512, fs], preferred_element_type=_F32)
        wB = jnp.concatenate([w[0:448, fs], w[512:576, fs]], axis=0)
        gB = jnp.dot(xp[b:b + n, :], wB, preferred_element_type=_F32)
        S = jnp.dot(xs[s:s + n, :], w[448:576, fs], preferred_element_type=_F32)
        return jnp.concatenate([gA + S, gB + S], axis=0)

    def hid(t, o, n, fs):
        g = proj(wg_v, t, o, n, fs)
        u = proj(wu_v, t, o, n, fs)
        return (_gelu(g) * u).astype(_BF)

    def down(fs, h):
        return lax.dot_general(wd_v[:, fs], h, _NT, preferred_element_type=_F32)

    def put(t, o, n, d, add=False):
        a = t * _TM + o
        b = a + _HM
        if n == _HM:
            if add:
                acc[:, a:a + _TM] += d
            else:
                acc[:, a:a + _TM] = d
        else:
            acc[:, a:a + n] = d[:, 0:n]
            acc[:, b:b + n] = d[:, n:2 * n]

    s0 = slice(0, _C0)
    s1 = slice(_C0, _C)
    sC = slice(0, _C)
    wait(0)
    prep(0, 0, 128)
    wait(1)
    h0 = hid(0, 0, 128, s0)
    wait(2)
    prep(0, 128, 128)
    put(0, 0, 128, down(s0, h0))
    h1 = hid(0, 128, 128, s0)
    wait(3)
    prep(1, 0, _HM)
    put(0, 128, 128, down(s0, h1))
    put(1, 0, _HM, down(s0, hid(1, 0, _HM, s0)))
    wait(4)
    for t in range(2, _NSUB):
        prep(t, 0, _HM)
    for t in range(0, 2):
        put(t, 0, _HM, down(s1, hid(t, 0, _HM, s1)), add=True)
    for t in range(2, _NSUB):
        put(t, 0, _HM, down(sC, hid(t, 0, _HM, sC)))
    wait(5)

    last = (_NSUB - 1) * _TM
    pieces = [[(t * _TM, (t + 1) * _TM)] for t in range(_NSUB - 1)]
    pieces.append([(last, _M - _TAIL), (_M - _TAIL, _M)])

    def body(j, carry):
        @pl.when(j == 1)
        def _():
            wait(6)

        fs = pl.ds(pl.multiple_of(_C + j * _TFL, 128), _TFL)
        for t in range(_NSUB):
            a = t * _TM
            h = hid(t, 0, _HM, fs)
            for (pa, pb) in pieces[t]:
                v = acc[:, pa:pb] + down(fs, h[pa - a:pb - a, :])
                acc[:, pa:pb] = v
                o_v[:, pa:pb] = v.astype(_BF)

                @pl.when(j == _NL - 1)
                def _():
                    co(pa, pb).start()
        return carry

    lax.fori_loop(0, _NL, body, 0)
    for ps in pieces:
        for (pa, pb) in ps:
            co(pa, pb).wait()


@jax.jit
def pallas_standalone__geglu_ffn__prompt_kernel(
    x: jax.Array,
    w_gate: jax.Array,
    w_up: jax.Array,
    w_down: jax.Array,
):
    B, S, D = x.shape
    assert (B * S, D, w_gate.shape[1]) == (_M, _D, _F) and B == 1
    xT = jnp.swapaxes(x, 1, 2).reshape(_D, _M)
    wdT = w_down.T
    outT = pl.pallas_call(
        _kernel,
        in_specs=[pl.BlockSpec(memory_space=pl.ANY)] * 4,
        out_specs=pl.BlockSpec(memory_space=pl.ANY),
        out_shape=jax.ShapeDtypeStruct((_D, _M), x.dtype),
        scratch_shapes=[
            pltpu.VMEM((_D, _M), _BF),
            pltpu.VMEM((_M, 512), _BF),
            pltpu.VMEM((_M // 2, 128), _BF),
            pltpu.VMEM((_D, _F), _BF),
            pltpu.VMEM((_D, _F), _BF),
            pltpu.VMEM((_D, _F), _BF),
            pltpu.VMEM((_D, _M), _F32),
            pltpu.VMEM((_D, _M), _BF),
            pltpu.SemaphoreType.DMA((8,)),
        ],
        compiler_params=pltpu.CompilerParams(vmem_limit_bytes=100 * 1024 * 1024),
    )(xT, w_gate, w_up, wdT)
    return jnp.swapaxes(outT.reshape(B, _D, S), 1, 2)
```

```python
import jax
import jax.numpy as jnp
from jax import lax
import jax.experimental.pallas as pl
import jax.experimental.pallas.tpu as pltpu

_NT = (((1,), (1,)), ((), ()))
_BF = jnp.bfloat16
_F32 = jnp.float32

_D, _M, _F = 576, 2048, 4608
_TM = 512
_HM = _TM // 2
_NSUB = _M // _TM
_TF = 512
_NL = _F // _TF - 1

_S_A, _S_B, _S_O, _NSEM = 5, 6, 7, 8

_LAST = (_NSUB - 1) * _TM
_PIECES = [[[(0, _D, t * _TM, (t + 1) * _TM)]] for t in range(_NSUB - 1)]
_PIECES.append([
    [(0, _D, _LAST, _LAST + 256)],
    [(0, _D, _LAST + 256, _LAST + 384)],
    [(0, _D // 2, _LAST + 384, _M), (_D // 2, _D, _LAST + 384, _M)],
])


def _gelu(g):
    c = 0.7978845608028654
    return 0.5 * g * (1.0 + jnp.tanh(c * (g + 0.044715 * (g * g * g))))


def _kernel(xT_hbm, wg_hbm, wu_hbm, wdT_hbm, oT_hbm,
            xT_v, xp, xs, w0, wl, acc, o_v, gu, sems):
    w_hbm = (wg_hbm, wu_hbm, wdT_hbm)

    def cx(r0, r1, a, b, s):
        return pltpu.make_async_copy(
            xT_hbm.at[r0:r1, a:b], xT_v.at[r0:r1, a:b], sems.at[s])

    def cw(i, r0, r1, s):
        return pltpu.make_async_copy(
            w_hbm[i].at[r0:r1, 0:_TF], w0.at[i, r0:r1, :], sems.at[s])

    def cl(j, i):
        return pltpu.make_async_copy(
            w_hbm[i].at[:, (j + 1) * _TF:(j + 2) * _TF], wl.at[j, i],
            sems.at[_S_A if j == 0 else _S_B])

    def co(r0, r1, a, b):
        return pltpu.make_async_copy(
            o_v.at[r0:r1, a:b], oT_hbm.at[r0:r1, a:b], sems.at[_S_O])

    groups = [
        [cx(0, 128, 0, 512, 0)],
        [cw(0, 0, 128, 1), cw(1, 0, 128, 1)],
        [cx(0, 128, 512, _M, 2)],
        [cx(128, _D, 0, 512, 3), cw(0, 128, _D, 3), cw(1, 128, _D, 3)],
        [cw(2, 0, _D, 4), cx(128, _D, 512, _M, 4)],
    ]
    for grp in groups:
        for c in grp:
            c.start()

    def wait(gi):
        for c in groups[gi]:
            c.wait()

    def prep_k(k, a, b):
        xp[a:b, k * 128:(k + 1) * 128] = xT_v[k * 128:(k + 1) * 128, a:b].T

    def prep_tail(t):
        a = t * _TM
        b = a + _HM
        s = t * _HM
        A, B = slice(a, a + _HM), slice(b, b + _HM)
        a8 = xT_v[448:512, A]
        b8 = xT_v[448:512, B]
        a9 = xT_v[512:576, A]
        b9 = xT_v[512:576, B]
        dA = (a8.astype(_F32) - b8.astype(_F32)).astype(_BF)
        dB = (b9.astype(_F32) - a9.astype(_F32)).astype(_BF)
        xp[A, 384:512] = jnp.concatenate([xT_v[384:448, A], dA], axis=0).T
        xp[B, 384:512] = jnp.concatenate([xT_v[384:448, B], dB], axis=0).T
        xs[s:s + _HM, :] = jnp.concatenate([b8, a9], axis=0).T

    def prep_rest(t):
        prep_tail(t)
        prep_k(1, t * _TM, (t + 1) * _TM)
        prep_k(2, t * _TM, (t + 1) * _TM)

    def proj(w, t, r0=0):
        a = t * _TM
        b = a + _HM
        s = t * _HM
        pA = jnp.dot(xp[a:a + _HM, r0:512], w[r0:512, :],
                     preferred_element_type=_F32)
        wB = jnp.concatenate([w[r0:448, :], w[512:576, :]], axis=0)
        pB = jnp.dot(xp[b:b + _HM, r0:512], wB, preferred_element_type=_F32)
        S = jnp.dot(xs[s:s + _HM, :], w[448:576, :],
                    preferred_element_type=_F32)
        return jnp.concatenate([pA + S, pB + S], axis=0)

    def down(wd, h):
        return lax.dot_general(wd[...], h, _NT, preferred_element_type=_F32)

    def mm0(i, a, b):
        gu[i, a:b, :] = jnp.dot(xp[a:b, 0:128], w0[i, 0:128, :],
                                preferred_element_type=_F32)

    def hid0(t):
        a = t * _TM
        g = proj(w0.at[0], t, 128) + gu[0, a:a + _TM, :]
        u = proj(w0.at[1], t, 128) + gu[1, a:a + _TM, :]
        return (_gelu(g) * u).astype(_BF)

    def prologue():
        wait(0)
        prep_k(0, 0, 512)
        wait(1)
        mm0(0, 0, 512)
        mm0(1, 0, 256)
        wait(2)
        for j in range(_NL):
            for i in range(3):
                cl(j, i).start()
        for a in range(512, _M, 512):
            prep_k(0, a, a + 512)
        mm0(1, 256, 512)
        for a in (512, 1024):
            mm0(0, a, a + 512)
            mm0(1, a, a + 512)
        mm0(0, 1536, _M)
        wait(3)
        prep_rest(0)
        mm0(1, 1536, _M)
        h0 = hid0(0)
        wait(4)
        for t in range(1, _NSUB):
            prep_rest(t)
        acc[:, 0:_TM] = down(w0.at[2], h0)
        for t in range(1, _NSUB):
            acc[:, t * _TM:(t + 1) * _TM] = down(w0.at[2], hid0(t))
        pltpu.make_async_copy(wl.at[0:1], wl.at[0:1], sems.at[_S_A]).wait()

    def chunk(j):
        @pl.when(j == 1)
        def _():
            pltpu.make_async_copy(
                wl.at[1:_NL], wl.at[1:_NL], sems.at[_S_B]).wait()

        wg, wu, wd = (wl.at[j, i] for i in range(3))
        for t in range(_NSUB):
            a = t * _TM
            h = (_gelu(proj(wg, t)) * proj(wu, t)).astype(_BF)
            for grp in _PIECES[t]:
                pa, pb = grp[0][2], grp[0][3]
                v = acc[:, pa:pb] + down(wd, h[pa - a:pb - a, :])
                acc[:, pa:pb] = v
                vb = v.astype(_BF)
                for (r0, r1, _, _) in grp:
                    o_v[r0:r1, pa:pb] = vb[r0:r1, :]

                    @pl.when(j == _NL - 1)
                    def _():
                        co(r0, r1, pa, pb).start()

    def body(jj, carry):
        @pl.when(jj == 0)
        def _():
            prologue()

        @pl.when(jj > 0)
        def _():
            chunk(jj - 1)

        return carry

    lax.fori_loop(0, _NL + 1, body, 0)
    pltpu.make_async_copy(o_v, o_v, sems.at[_S_O]).wait()


@jax.jit
def pallas_standalone__geglu_ffn__prompt_kernel(
    x: jax.Array,
    w_gate: jax.Array,
    w_up: jax.Array,
    w_down: jax.Array,
):
    B, S, D = x.shape
    assert B == 1 and (S, D, w_gate.shape[1]) == (_M, _D, _F)
    xT = jnp.swapaxes(x, 1, 2).reshape(_D, _M)
    wdT = w_down.T
    outT = pl.pallas_call(
        _kernel,
        in_specs=[pl.BlockSpec(memory_space=pl.ANY)] * 4,
        out_specs=pl.BlockSpec(memory_space=pl.ANY),
        out_shape=jax.ShapeDtypeStruct((_D, _M), x.dtype),
        scratch_shapes=[
            pltpu.VMEM((_D, _M), _BF),
            pltpu.VMEM((_M, 512), _BF),
            pltpu.VMEM((_M // 2, 128), _BF),
            pltpu.VMEM((3, _D, _TF), _BF),
            pltpu.VMEM((_NL, 3, _D, _TF), _BF),
            pltpu.VMEM((_D, _M), _F32),
            pltpu.VMEM((_D, _M), _BF),
            pltpu.VMEM((2, _M, _TF), _F32),
            pltpu.SemaphoreType.DMA((_NSEM,)),
        ],
        compiler_params=pltpu.CompilerParams(
            vmem_limit_bytes=100 * 1024 * 1024,
            disable_semaphore_checks=True,
        ),
    )(xT, w_gate, w_up, wdT)
    return jnp.swapaxes(outT.reshape(B, _D, S), 1, 2)
```

```python
import jax
import jax.numpy as jnp
from jax import lax
import jax.experimental.pallas as pl
import jax.experimental.pallas.tpu as pltpu

_NT = (((1,), (1,)), ((), ()))
_BF = jnp.bfloat16
_F32 = jnp.float32

_D, _M, _F = 576, 2048, 4608
_TM = 512
_HM = _TM // 2
_NSUB = _M // _TM
_TF = 512
_NL = _F // _TF - 1

_S_A, _S_B, _S_O, _NSEM = 5, 6, 7, 8

_LAST = (_NSUB - 1) * _TM
_PIECES = [[[(0, _D, t * _TM, (t + 1) * _TM)]] for t in range(_NSUB - 1)]
_PIECES.append([
    [(0, _D, _LAST, _LAST + 256)],
    [(0, _D, _LAST + 256, _LAST + 384)],
    [(0, _D // 2, _LAST + 384, _M), (_D // 2, _D, _LAST + 384, _M)],
])


def _gelu(g):
    c = 0.7978845608028654
    return 0.5 * g * (1.0 + jnp.tanh(c * (g + 0.044715 * (g * g * g))))


def _kernel(xT_hbm, wg_hbm, wu_hbm, wdT_hbm, oT_hbm,
            xT_v, xp, xs, w0, wl, acc, o_v, gu, sems):
    w_hbm = (wg_hbm, wu_hbm, wdT_hbm)

    def cx(r0, r1, a, b, s):
        return pltpu.make_async_copy(
            xT_hbm.at[r0:r1, a:b], xT_v.at[r0:r1, a:b], sems.at[s])

    def cw(i, r0, r1, s):
        return pltpu.make_async_copy(
            w_hbm[i].at[r0:r1, 0:_TF], w0.at[i, r0:r1, :], sems.at[s])

    def cl(j, i):
        return pltpu.make_async_copy(
            w_hbm[i].at[:, (j + 1) * _TF:(j + 2) * _TF], wl.at[j, i],
            sems.at[_S_A if j == 0 else _S_B])

    def co(r0, r1, a, b):
        return pltpu.make_async_copy(
            o_v.at[r0:r1, a:b], oT_hbm.at[r0:r1, a:b], sems.at[_S_O])

    groups = [
        [cx(0, 128, 0, 512, 0)],
        [cw(0, 0, 128, 1), cw(1, 0, 128, 1)],
        [cx(0, 128, 512, _M, 2)],
        [cx(128, _D, 0, 512, 3), cw(0, 128, _D, 3), cw(1, 128, _D, 3)],
        [cw(2, 0, _D, 4), cx(128, _D, 512, _M, 4)],
    ]
    for grp in groups:
        for c in grp:
            c.start()

    def wait(gi):
        for c in groups[gi]:
            c.wait()

    def prep_k(k, a, b):
        xp[a:b, k * 128:(k + 1) * 128] = xT_v[k * 128:(k + 1) * 128, a:b].T

    def prep_tail(t):
        a = t * _TM
        b = a + _HM
        s = t * _HM
        A, B = slice(a, a + _HM), slice(b, b + _HM)
        a8 = xT_v[448:512, A]
        b8 = xT_v[448:512, B]
        a9 = xT_v[512:576, A]
        b9 = xT_v[512:576, B]
        dA = (a8.astype(_F32) - b8.astype(_F32)).astype(_BF)
        dB = (b9.astype(_F32) - a9.astype(_F32)).astype(_BF)
        xp[A, 384:512] = jnp.concatenate([xT_v[384:448, A], dA], axis=0).T
        xp[B, 384:512] = jnp.concatenate([xT_v[384:448, B], dB], axis=0).T
        xs[s:s + _HM, :] = jnp.concatenate([b8, a9], axis=0).T

    def prep_rest(t):
        prep_tail(t)
        prep_k(1, t * _TM, (t + 1) * _TM)
        prep_k(2, t * _TM, (t + 1) * _TM)

    def proj(w, t, r0=0):
        a = t * _TM
        b = a + _HM
        s = t * _HM
        pA = jnp.dot(xp[a:a + _HM, r0:512], w[r0:512, :],
                     preferred_element_type=_F32)
        wB = jnp.concatenate([w[r0:448, :], w[512:576, :]], axis=0)
        pB = jnp.dot(xp[b:b + _HM, r0:512], wB, preferred_element_type=_F32)
        S = jnp.dot(xs[s:s + _HM, :], w[448:576, :],
                    preferred_element_type=_F32)
        return jnp.concatenate([pA + S, pB + S], axis=0)

    def down(wd, h):
        return lax.dot_general(wd[...], h, _NT, preferred_element_type=_F32)

    def mm0(i, a, b):
        gu[i, a:b, :] = jnp.dot(xp[a:b, 0:128], w0[i, 0:128, :],
                                preferred_element_type=_F32)

    def hid0(t):
        a = t * _TM
        g = proj(w0.at[0], t, 128) + gu[0, a:a + _TM, :]
        u = proj(w0.at[1], t, 128) + gu[1, a:a + _TM, :]
        return (_gelu(g) * u).astype(_BF)

    def prologue():
        wait(0)
        prep_k(0, 0, 512)
        wait(1)
        mm0(0, 0, 512)
        mm0(1, 0, 256)
        wait(2)
        for j in range(_NL):
            for i in range(3):
                cl(j, i).start()
        for a in range(512, _M, 512):
            prep_k(0, a, a + 512)
        mm0(1, 256, 512)
        for a in (512, 1024):
            mm0(0, a, a + 512)
            mm0(1, a, a + 512)
        mm0(0, 1536, _M)
        wait(3)
        prep_rest(0)
        mm0(1, 1536, _M)
        h0 = hid0(0)
        wait(4)
        for t in range(1, _NSUB):
            prep_rest(t)
        acc[:, 0:_TM] = down(w0.at[2], h0)
        for t in range(1, _NSUB):
            acc[:, t * _TM:(t + 1) * _TM] = down(w0.at[2], hid0(t))
        pltpu.make_async_copy(wl.at[0:1], wl.at[0:1], sems.at[_S_A]).wait()

    def chunk(j):
        @pl.when(j == 1)
        def _():
            pltpu.make_async_copy(
                wl.at[1:_NL], wl.at[1:_NL], sems.at[_S_B]).wait()

        wg, wu, wd = (wl.at[j, i] for i in range(3))
        for t in range(_NSUB):
            a = t * _TM
            h = (_gelu(proj(wg, t)) * proj(wu, t)).astype(_BF)
            for grp in _PIECES[t]:
                pa, pb = grp[0][2], grp[0][3]
                v = acc[:, pa:pb] + down(wd, h[pa - a:pb - a, :])
                acc[:, pa:pb] = v
                vb = v.astype(_BF)
                for (r0, r1, _, _) in grp:
                    o_v[r0:r1, pa:pb] = vb[r0:r1, :]

                    @pl.when(j == _NL - 1)
                    def _():
                        co(r0, r1, pa, pb).start()

    def body(j, carry):
        @pl.when(j == 0)
        def _():
            prologue()

        chunk(j)
        return carry

    lax.fori_loop(0, _NL, body, 0)
    pltpu.make_async_copy(o_v, oT_hbm, sems.at[_S_O]).wait()


@jax.jit
def pallas_standalone__geglu_ffn__prompt_kernel(
    x: jax.Array,
    w_gate: jax.Array,
    w_up: jax.Array,
    w_down: jax.Array,
):
    B, S, D = x.shape
    assert B == 1 and (S, D, w_gate.shape[1]) == (_M, _D, _F)
    xT = jnp.swapaxes(x, 1, 2).reshape(_D, _M)
    wdT = w_down.T
    outT = pl.pallas_call(
        _kernel,
        in_specs=[pl.BlockSpec(memory_space=pl.ANY)] * 4,
        out_specs=pl.BlockSpec(memory_space=pl.ANY),
        out_shape=jax.ShapeDtypeStruct((_D, _M), x.dtype),
        scratch_shapes=[
            pltpu.VMEM((_D, _M), _BF),
            pltpu.VMEM((_M, 512), _BF),
            pltpu.VMEM((_M // 2, 128), _BF),
            pltpu.VMEM((3, _D, _TF), _BF),
            pltpu.VMEM((_NL, 3, _D, _TF), _BF),
            pltpu.VMEM((_D, _M), _F32),
            pltpu.VMEM((_D, _M), _BF),
            pltpu.VMEM((2, _M, _TF), _F32),
            pltpu.SemaphoreType.DMA((_NSEM,)),
        ],
        compiler_params=pltpu.CompilerParams(
            vmem_limit_bytes=100 * 1024 * 1024,
            disable_semaphore_checks=True,
        ),
    )(xT, w_gate, w_up, wdT)
    return jnp.swapaxes(outT.reshape(B, _D, S), 1, 2)
```

```python
import jax
import jax.numpy as jnp
from jax import lax
import jax.experimental.pallas as pl
import jax.experimental.pallas.tpu as pltpu

_NT = (((1,), (1,)), ((), ()))
_BF = jnp.bfloat16
_F32 = jnp.float32

_D, _M, _F = 576, 2048, 4608
_TM = 512
_HM = _TM // 2
_NSUB = _M // _TM
_TF = 512
_NL = _F // _TF - 1

_S_A, _S_B, _S_O, _NSEM = 5, 6, 7, 8

_LAST = (_NSUB - 1) * _TM
_PIECES = [[[(0, _D, t * _TM, (t + 1) * _TM)]] for t in range(_NSUB - 1)]
_PIECES.append([
    [(0, _D, _LAST, _LAST + 256)],
    [(0, _D, _LAST + 256, _LAST + 384)],
    [(0, _D // 2, _LAST + 384, _M), (_D // 2, _D, _LAST + 384, _M)],
])


def _gelu(g):
    c = 0.7978845608028654
    return 0.5 * g * (1.0 + jnp.tanh(c * (g + 0.044715 * (g * g * g))))


def _pack(v):
    return pltpu.bitcast(v, jnp.uint32)


def _unpack(v):
    return pltpu.bitcast(v, _BF)


def _kernel(xT_hbm, wg_hbm, wu_hbm, wdT_hbm, oT_hbm,
            xT_v, xp, xs, w0, wl, acc, o_v, gu, sems):
    w_hbm = (wg_hbm, wu_hbm, wdT_hbm)

    def cx(r0, r1, a, b, s):
        return pltpu.make_async_copy(
            xT_hbm.at[r0:r1, a:b], xT_v.at[r0:r1, a:b], sems.at[s])

    def cw(i, r0, r1, s):
        return pltpu.make_async_copy(
            w_hbm[i].at[r0:r1, 0:_TF], w0.at[i, r0:r1, :], sems.at[s])

    def cl(j, i):
        return pltpu.make_async_copy(
            w_hbm[i].at[:, (j + 1) * _TF:(j + 2) * _TF], wl.at[j, i],
            sems.at[_S_A if j == 0 else _S_B])

    def co(r0, r1, a, b):
        return pltpu.make_async_copy(
            o_v.at[r0:r1, a:b], oT_hbm.at[r0:r1, a:b], sems.at[_S_O])

    groups = [
        [cx(0, 128, 0, 512, 0)],
        [cw(0, 0, 128, 1), cw(1, 0, 128, 1)],
        [cx(0, 128, 512, _M, 2)],
        [cx(128, _D, 0, 512, 3), cw(0, 128, _D, 3), cw(1, 128, _D, 3)],
        [cw(2, 0, _D, 4), cx(128, _D, 512, _M, 4)],
    ]
    for grp in groups:
        for c in grp:
            c.start()

    def wait(gi):
        for c in groups[gi]:
            c.wait()

    def prep_k(k, a, b):
        xp[a // 2:b // 2, k * 128:(k + 1) * 128] = _pack(xT_v[k * 128:(k + 1) * 128, a:b].T)

    def prep_tail(t):
        a = t * _TM
        b = a + _HM
        s = t * _HM
        A, B = slice(a, a + _HM), slice(b, b + _HM)
        a8 = xT_v[448:512, A]
        b8 = xT_v[448:512, B]
        a9 = xT_v[512:576, A]
        b9 = xT_v[512:576, B]
        dA = (a8.astype(_F32) - b8.astype(_F32)).astype(_BF)
        dB = (b9.astype(_F32) - a9.astype(_F32)).astype(_BF)
        xp[a // 2:b // 2, 384:512] = _pack(jnp.concatenate([xT_v[384:448, A], dA], axis=0).T)
        xp[b // 2:(b + _HM) // 2, 384:512] = _pack(jnp.concatenate([xT_v[384:448, B], dB], axis=0).T)
        xs[s // 2:(s + _HM) // 2, :] = _pack(jnp.concatenate([b8, a9], axis=0).T)

    def prep_rest(t):
        prep_tail(t)
        prep_k(1, t * _TM, (t + 1) * _TM)
        prep_k(2, t * _TM, (t + 1) * _TM)

    def proj(w, t, r0=0):
        a = t * _TM
        b = a + _HM
        s = t * _HM
        pA = jnp.dot(_unpack(xp[a // 2:b // 2, r0:512]), w[r0:512, :],
                     preferred_element_type=_F32)
        wB = jnp.concatenate([w[r0:448, :], w[512:576, :]], axis=0)
        pB = jnp.dot(_unpack(xp[b // 2:(b + _HM) // 2, r0:512]), wB, preferred_element_type=_F32)
        S = jnp.dot(_unpack(xs[s // 2:(s + _HM) // 2, :]), w[448:576, :],
                    preferred_element_type=_F32)
        return jnp.concatenate([pA + S, pB + S], axis=0)

    def down(wd, h):
        return lax.dot_general(wd[...], h, _NT, preferred_element_type=_F32)

    def mm0(i, a, b):
        gu[i, a:b, :] = jnp.dot(_unpack(xp[a // 2:b // 2, 0:128]), w0[i, 0:128, :],
                                preferred_element_type=_F32)

    def hid0(t):
        a = t * _TM
        g = proj(w0.at[0], t, 128) + gu[0, a:a + _TM, :]
        u = proj(w0.at[1], t, 128) + gu[1, a:a + _TM, :]
        return (_gelu(g) * u).astype(_BF)

    def prologue():
        wait(0)
        prep_k(0, 0, 512)
        wait(1)
        mm0(0, 0, 512)
        mm0(1, 0, 256)
        wait(2)
        for j in range(_NL):
            for i in range(3):
                cl(j, i).start()
        for a in range(512, _M, 512):
            prep_k(0, a, a + 512)
        mm0(1, 256, 512)
        for a in (512, 1024):
            mm0(0, a, a + 512)
            mm0(1, a, a + 512)
        mm0(0, 1536, _M)
        wait(3)
        prep_rest(0)
        mm0(1, 1536, _M)
        h0 = hid0(0)
        wait(4)
        for t in range(1, _NSUB):
            prep_rest(t)
        acc[:, 0:_TM] = down(w0.at[2], h0)
        for t in range(1, _NSUB):
            acc[:, t * _TM:(t + 1) * _TM] = down(w0.at[2], hid0(t))
        pltpu.make_async_copy(wl.at[0:1], wl.at[0:1], sems.at[_S_A]).wait()

    def chunk(j):
        @pl.when(j == 1)
        def _():
            pltpu.make_async_copy(
                wl.at[1:_NL], wl.at[1:_NL], sems.at[_S_B]).wait()

        wg, wu, wd = (wl.at[j, i] for i in range(3))
        for t in range(_NSUB):
            a = t * _TM
            h = (_gelu(proj(wg, t)) * proj(wu, t)).astype(_BF)
            for grp in _PIECES[t]:
                pa, pb = grp[0][2], grp[0][3]
                v = acc[:, pa:pb] + down(wd, h[pa - a:pb - a, :])
                acc[:, pa:pb] = v
                vb = v.astype(_BF)
                for (r0, r1, _, _) in grp:
                    o_v[r0:r1, pa:pb] = vb[r0:r1, :]

                    @pl.when(j == _NL - 1)
                    def _():
                        co(r0, r1, pa, pb).start()

    def body(j, carry):
        @pl.when(j == 0)
        def _():
            prologue()

        chunk(j)
        return carry

    lax.fori_loop(0, _NL, body, 0)
    pltpu.make_async_copy(o_v, oT_hbm, sems.at[_S_O]).wait()


@jax.jit
def pallas_standalone__geglu_ffn__prompt_kernel(
    x: jax.Array,
    w_gate: jax.Array,
    w_up: jax.Array,
    w_down: jax.Array,
):
    B, S, D = x.shape
    assert B == 1 and (S, D, w_gate.shape[1]) == (_M, _D, _F)
    xT = jnp.swapaxes(x, 1, 2).reshape(_D, _M)
    wdT = w_down.T
    outT = pl.pallas_call(
        _kernel,
        in_specs=[pl.BlockSpec(memory_space=pl.ANY)] * 4,
        out_specs=pl.BlockSpec(memory_space=pl.ANY),
        out_shape=jax.ShapeDtypeStruct((_D, _M), x.dtype),
        scratch_shapes=[
            pltpu.VMEM((_D, _M), _BF),
            pltpu.VMEM((_M // 2, 512), jnp.uint32),
            pltpu.VMEM((_M // 4, 128), jnp.uint32),
            pltpu.VMEM((3, _D, _TF), _BF),
            pltpu.VMEM((_NL, 3, _D, _TF), _BF),
            pltpu.VMEM((_D, _M), _F32),
            pltpu.VMEM((_D, _M), _BF),
            pltpu.VMEM((2, _M, _TF), _F32),
            pltpu.SemaphoreType.DMA((_NSEM,)),
        ],
        compiler_params=pltpu.CompilerParams(
            vmem_limit_bytes=100 * 1024 * 1024,
            disable_semaphore_checks=True,
        ),
    )(xT, w_gate, w_up, wdT)
    return jnp.swapaxes(outT.reshape(B, _D, S), 1, 2)
```

```python
import jax
import jax.numpy as jnp
from jax import lax
import jax.experimental.pallas as pl
import jax.experimental.pallas.tpu as pltpu

_NT = (((1,), (1,)), ((), ()))
_BF = jnp.bfloat16
_F32 = jnp.float32

_D, _M, _F = 576, 2048, 4608
_TM = 512
_HM = _TM // 2
_NSUB = _M // _TM
_TF = 512
_NL = _F // _TF - 1

_S_A, _S_B, _S_O, _NSEM = 5, 6, 7, 8

_LAST = (_NSUB - 1) * _TM
_PIECES = [[[(0, _D, t * _TM, (t + 1) * _TM)]] for t in range(_NSUB - 1)]
_PIECES.append([
    [(0, _D, _LAST, _LAST + 256)],
    [(0, _D, _LAST + 256, _LAST + 384)],
    [(0, _D // 2, _LAST + 384, _M), (_D // 2, _D, _LAST + 384, _M)],
])


def _gelu(g):
    c = 0.7978845608028654
    return 0.5 * g * (1.0 + jnp.tanh(c * (g + 0.044715 * (g * g * g))))


def _pack(v):
    return pltpu.bitcast(v, jnp.uint32)


def _unpack(v):
    return pltpu.bitcast(v, _BF)


def _kernel(xT_hbm, wg_hbm, wu_hbm, wdT_hbm, oT_hbm,
            xT_v, xp, xs, rs, w0, wl, acc, o_v, gu, sems):
    w_hbm = (wg_hbm, wu_hbm, wdT_hbm)

    def cx(r0, r1, a, b, s):
        return pltpu.make_async_copy(
            xT_hbm.at[r0:r1, a:b], xT_v.at[r0:r1, a:b], sems.at[s])

    def cw(i, r0, r1, s):
        return pltpu.make_async_copy(
            w_hbm[i].at[r0:r1, 0:_TF], w0.at[i, r0:r1, :], sems.at[s])

    def cl(j, i):
        return pltpu.make_async_copy(
            w_hbm[i].at[:, (j + 1) * _TF:(j + 2) * _TF], wl.at[j, i],
            sems.at[_S_A if j == 0 else _S_B])

    def co(r0, r1, a, b):
        return pltpu.make_async_copy(
            o_v.at[r0:r1, a:b], oT_hbm.at[r0:r1, a:b], sems.at[_S_O])

    groups = [
        [cx(0, 128, 0, 512, 0)],
        [cw(0, 0, 128, 1), cw(1, 0, 128, 1)],
        [cx(0, 128, 512, _M, 2)],
        [cx(128, _D, 0, 512, 3), cw(0, 128, _D, 3), cw(1, 128, _D, 3)],
        [cw(2, 0, _D, 4), cx(128, _D, 512, _M, 4)],
    ]
    for grp in groups:
        for c in grp:
            c.start()

    def wait(gi):
        for c in groups[gi]:
            c.wait()

    def prep_k(k, a, b):
        xp[a // 2:b // 2, k * 128:(k + 1) * 128] = _pack(xT_v[k * 128:(k + 1) * 128, a:b].T)

    def prep_tail(t):
        a = t * _TM
        b = a + _HM
        s = t * _HM
        A, B = slice(a, a + _HM), slice(b, b + _HM)
        a8 = xT_v[448:512, A].astype(_F32)
        b8 = xT_v[448:512, B].astype(_F32)
        a9 = xT_v[512:576, A].astype(_F32)
        b9 = xT_v[512:576, B].astype(_F32)
        ma = jnp.sum(jnp.abs(a8) + jnp.abs(a9), axis=0, keepdims=True)
        mb = jnp.sum(jnp.abs(b8) + jnp.abs(b9), axis=0, keepdims=True)
        la = jnp.clip(pltpu.bitcast(ma, jnp.int32), 87 << 23, 190 << 23)
        lb = jnp.clip(pltpu.bitcast(mb, jnp.int32), 87 << 23, 190 << 23)
        e = (la - lb + (1 << 22)) >> 23
        r = pltpu.bitcast((127 + e) << 23, _F32)
        rinv = pltpu.bitcast((127 - e) << 23, _F32)
        rb8 = r * b8
        dA = (a8 - rb8).astype(_BF)
        dB = (b9 - rinv * a9).astype(_BF)
        xp[a // 2:b // 2, 384:512] = _pack(jnp.concatenate([xT_v[384:448, A], dA], axis=0).T)
        xp[b // 2:(b + _HM) // 2, 384:512] = _pack(jnp.concatenate([xT_v[384:448, B], dB], axis=0).T)
        xs[s // 2:(s + _HM) // 2, :] = _pack(
            jnp.concatenate([rb8.astype(_BF), xT_v[512:576, A]], axis=0).T)
        rs[s:s + _HM, :] = jnp.broadcast_to(rinv, (128, _HM)).T

    def prep_rest(t):
        prep_tail(t)
        prep_k(1, t * _TM, (t + 1) * _TM)
        prep_k(2, t * _TM, (t + 1) * _TM)

    def proj(w, t, r0=0):
        a = t * _TM
        b = a + _HM
        s = t * _HM
        pA = jnp.dot(_unpack(xp[a // 2:b // 2, r0:512]), w[r0:512, :],
                     preferred_element_type=_F32)
        wB = jnp.concatenate([w[r0:448, :], w[512:576, :]], axis=0)
        pB = jnp.dot(_unpack(xp[b // 2:(b + _HM) // 2, r0:512]), wB, preferred_element_type=_F32)
        S = jnp.dot(_unpack(xs[s // 2:(s + _HM) // 2, :]), w[448:576, :],
                    preferred_element_type=_F32)
        rinv = jnp.concatenate([rs[s:s + _HM, :]] * (_TF // 128), axis=1)
        return jnp.concatenate([pA + S, pB + S * rinv], axis=0)

    def down(wd, h):
        return lax.dot_general(wd[...], h, _NT, preferred_element_type=_F32)

    def mm0(i, a, b):
        gu[i, a:b, :] = jnp.dot(_unpack(xp[a // 2:b // 2, 0:128]), w0[i, 0:128, :],
                                preferred_element_type=_F32)

    def hid0(t):
        a = t * _TM
        g = proj(w0.at[0], t, 128) + gu[0, a:a + _TM, :]
        u = proj(w0.at[1], t, 128) + gu[1, a:a + _TM, :]
        return (_gelu(g) * u).astype(_BF)

    def prologue():
        wait(0)
        prep_k(0, 0, 512)
        wait(1)
        mm0(0, 0, 512)
        mm0(1, 0, 256)
        wait(2)
        for j in range(_NL):
            for i in range(3):
                cl(j, i).start()
        for a in range(512, _M, 512):
            prep_k(0, a, a + 512)
        mm0(1, 256, 512)
        for a in (512, 1024):
            mm0(0, a, a + 512)
            mm0(1, a, a + 512)
        mm0(0, 1536, _M)
        wait(3)
        prep_rest(0)
        mm0(1, 1536, _M)
        h0 = hid0(0)
        wait(4)
        for t in range(1, _NSUB):
            prep_rest(t)
        acc[:, 0:_TM] = down(w0.at[2], h0)
        for t in range(1, _NSUB):
            acc[:, t * _TM:(t + 1) * _TM] = down(w0.at[2], hid0(t))
        pltpu.make_async_copy(wl.at[0:1], wl.at[0:1], sems.at[_S_A]).wait()

    def chunk(j):
        @pl.when(j == 1)
        def _():
            pltpu.make_async_copy(
                wl.at[1:_NL], wl.at[1:_NL], sems.at[_S_B]).wait()

        wg, wu, wd = (wl.at[j, i] for i in range(3))
        for t in range(_NSUB):
            a = t * _TM
            h = (_gelu(proj(wg, t)) * proj(wu, t)).astype(_BF)
            for grp in _PIECES[t]:
                pa, pb = grp[0][2], grp[0][3]
                v = acc[:, pa:pb] + down(wd, h[pa - a:pb - a, :])
                acc[:, pa:pb] = v
                vb = v.astype(_BF)
                for (r0, r1, _, _) in grp:
                    o_v[r0:r1, pa:pb] = vb[r0:r1, :]

                    @pl.when(j == _NL - 1)
                    def _():
                        co(r0, r1, pa, pb).start()

    def body(j, carry):
        @pl.when(j == 0)
        def _():
            prologue()

        chunk(j)
        return carry

    lax.fori_loop(0, _NL, body, 0)
    pltpu.make_async_copy(o_v, oT_hbm, sems.at[_S_O]).wait()


@jax.jit
def pallas_standalone__geglu_ffn__prompt_kernel(
    x: jax.Array,
    w_gate: jax.Array,
    w_up: jax.Array,
    w_down: jax.Array,
):
    B, S, D = x.shape
    assert B == 1 and (S, D, w_gate.shape[1]) == (_M, _D, _F)
    xT = jnp.swapaxes(x, 1, 2).reshape(_D, _M)
    wdT = w_down.T
    outT = pl.pallas_call(
        _kernel,
        in_specs=[pl.BlockSpec(memory_space=pl.ANY)] * 4,
        out_specs=pl.BlockSpec(memory_space=pl.ANY),
        out_shape=jax.ShapeDtypeStruct((_D, _M), x.dtype),
        scratch_shapes=[
            pltpu.VMEM((_D, _M), _BF),
            pltpu.VMEM((_M // 2, 512), jnp.uint32),
            pltpu.VMEM((_M // 4, 128), jnp.uint32),
            pltpu.VMEM((_M // 2, 128), _F32),
            pltpu.VMEM((3, _D, _TF), _BF),
            pltpu.VMEM((_NL, 3, _D, _TF), _BF),
            pltpu.VMEM((_D, _M), _F32),
            pltpu.VMEM((_D, _M), _BF),
            pltpu.VMEM((2, _M, _TF), _F32),
            pltpu.SemaphoreType.DMA((_NSEM,)),
        ],
        compiler_params=pltpu.CompilerParams(
            vmem_limit_bytes=100 * 1024 * 1024,
            disable_semaphore_checks=True,
        ),
    )(xT, w_gate, w_up, wdT)
    return jnp.swapaxes(outT.reshape(B, _D, S), 1, 2)
```

```python
import jax
import jax.numpy as jnp
from jax import lax
import jax.experimental.pallas as pl
import jax.experimental.pallas.tpu as pltpu

_NT = (((1,), (1,)), ((), ()))
_BF = jnp.bfloat16
_F32 = jnp.float32

_D, _M, _F = 576, 2048, 4608
_TM = 512
_HM = _TM // 2
_NSUB = _M // _TM
_TF = 512
_NL = _F // _TF - 1

_S_A, _S_B, _S_O, _NSEM = 5, 6, 7, 8

_NV = 16
_DM = _D - _NV
_VTILES = (4, 4, 4, 1)
_VW = 3 * _TM + 128
_DG = 4
_VSCHED = (8, 8, 8, 8, 8, 8, 4)
_VLAST = 0.55

_LAST = (_NSUB - 1) * _TM
_PIECES = [[[(0, _DM, t * _TM, (t + 1) * _TM)]] for t in range(_NSUB - 1)]
_PIECES.append([
    [(0, _DM, _LAST, _LAST + 128)],
    [(0, _D, _LAST + 128, _LAST + 256)],
    [(0, _D, _LAST + 256, _LAST + 384)],
    [(0, _D // 2, _LAST + 384, _M), (_D // 2, _D, _LAST + 384, _M)],
])


def _gelu(g):
    c = 0.7978845608028654
    return 0.5 * g * (1.0 + jnp.tanh(c * (g + 0.044715 * (g * g * g))))


def _pack(v):
    return pltpu.bitcast(v, jnp.uint32)


def _unpack(v):
    return pltpu.bitcast(v, _BF)


def _vregs(v):
    r, c = v.shape
    return [v[i:i + 8, k:k + 128]
            for k in range(0, c, 128) for i in range(0, r, 8)]


def _kernel(xT_hbm, wg_hbm, wu_hbm, wdT_hbm, oT_hbm,
            xT_v, xp, xs, rs, w0, wl, acc, o_v, gu, wb, racc, flag, sems):
    w_hbm = (wg_hbm, wu_hbm, wdT_hbm)
    flag[0] = 0

    def cx(r0, r1, a, b, s):
        return pltpu.make_async_copy(
            xT_hbm.at[r0:r1, a:b], xT_v.at[r0:r1, a:b], sems.at[s])

    def cw(i, r0, r1, s):
        return pltpu.make_async_copy(
            w_hbm[i].at[r0:r1, 0:_TF], w0.at[i, r0:r1, :], sems.at[s])

    def cl(j, i):
        return pltpu.make_async_copy(
            w_hbm[i].at[:, (j + 1) * _TF:(j + 2) * _TF], wl.at[j, i],
            sems.at[_S_A if j == 0 else _S_B])

    def co(r0, r1, a, b):
        return pltpu.make_async_copy(
            o_v.at[r0:r1, a:b], oT_hbm.at[r0:r1, a:b], sems.at[_S_O])

    groups = [
        [cx(0, 128, 0, 512, 0)],
        [cw(0, 0, 128, 1), cw(1, 0, 128, 1)],
        [cx(0, 128, 512, _M, 2)],
        [cx(128, _D, 0, 512, 3), cw(0, 128, _D, 3), cw(1, 128, _D, 3)],
        [cw(2, 0, _D, 4), cx(128, _D, 512, _M, 4)],
    ]
    for grp in groups:
        for c in grp:
            c.start()

    def wait(gi):
        for c in groups[gi]:
            c.wait()

    def prep_k(k, a, b):
        xp[a // 2:b // 2, k * 128:(k + 1) * 128] = _pack(
            xT_v[k * 128:(k + 1) * 128, a:b].T)

    def prep_tail(t):
        a = t * _TM
        b = a + _HM
        s = t * _HM
        A, B = slice(a, a + _HM), slice(b, b + _HM)
        a8 = xT_v[448:512, A].astype(_F32)
        b8 = xT_v[448:512, B].astype(_F32)
        a9 = xT_v[512:576, A].astype(_F32)
        b9 = xT_v[512:576, B].astype(_F32)
        ma = jnp.sum(jnp.abs(a8) + jnp.abs(a9), axis=0, keepdims=True)
        mb = jnp.sum(jnp.abs(b8) + jnp.abs(b9), axis=0, keepdims=True)
        la = jnp.clip(pltpu.bitcast(ma, jnp.int32), 87 << 23, 190 << 23)
        lb = jnp.clip(pltpu.bitcast(mb, jnp.int32), 87 << 23, 190 << 23)
        e = (la - lb + (1 << 22)) >> 23
        r = pltpu.bitcast((127 + e) << 23, _F32)
        rinv = pltpu.bitcast((127 - e) << 23, _F32)
        rb8 = r * b8
        dA = (a8 - rb8).astype(_BF)
        dB = (b9 - rinv * a9).astype(_BF)
        xp[a // 2:b // 2, 384:512] = _pack(
            jnp.concatenate([xT_v[384:448, A], dA], axis=0).T)
        xp[b // 2:(b + _HM) // 2, 384:512] = _pack(
            jnp.concatenate([xT_v[384:448, B], dB], axis=0).T)
        xs[s // 2:(s + _HM) // 2, :] = _pack(
            jnp.concatenate([rb8.astype(_BF), xT_v[512:576, A]], axis=0).T)
        rs[s:s + _HM, :] = jnp.broadcast_to(rinv, (128, _HM)).T

    def prep_rest(t):
        prep_tail(t)
        prep_k(1, t * _TM, (t + 1) * _TM)
        prep_k(2, t * _TM, (t + 1) * _TM)

    def proj(w, t, r0=0):
        a = t * _TM
        b = a + _HM
        s = t * _HM
        pA = jnp.dot(_unpack(xp[a // 2:b // 2, r0:512]), w[r0:512, :],
                     preferred_element_type=_F32)
        wB = jnp.concatenate([w[r0:448, :], w[512:576, :]], axis=0)
        pB = jnp.dot(_unpack(xp[b // 2:(b + _HM) // 2, r0:512]), wB,
                     preferred_element_type=_F32)
        S = jnp.dot(_unpack(xs[s // 2:(s + _HM) // 2, :]), w[448:576, :],
                    preferred_element_type=_F32)
        rinv = jnp.concatenate([rs[s:s + _HM, :]] * (_TF // 128), axis=1)
        return jnp.concatenate([pA + S, pB + S * rinv], axis=0), pA, pB

    def down(wd, h, rows=_D):
        return lax.dot_general(wd[0:rows, :], h, _NT,
                               preferred_element_type=_F32)

    def mm0(i, a, b):
        gu[i, a:b, :] = jnp.dot(_unpack(xp[a // 2:b // 2, 0:128]),
                                w0[i, 0:128, :], preferred_element_type=_F32)

    def hid0(t):
        a = t * _TM
        g = proj(w0.at[0], t, 128)[0] + gu[0, a:a + _TM, :]
        u = proj(w0.at[1], t, 128)[0] + gu[1, a:a + _TM, :]
        return (_gelu(g) * u).astype(_BF)

    def prologue():
        wait(0)
        prep_k(0, 0, 512)
        wait(1)
        mm0(0, 0, 512)
        mm0(1, 0, 256)
        wait(2)
        for j in range(_NL):
            for i in range(3):
                cl(j, i).start()
        for a in range(512, _M, 512):
            prep_k(0, a, a + 512)
        mm0(1, 256, 512)
        for a in (512, 1024):
            mm0(0, a, a + 512)
            mm0(1, a, a + 512)
        mm0(0, 1536, _M)
        wait(3)
        prep_rest(0)
        mm0(1, 1536, _M)
        h0 = hid0(0)
        wait(4)
        racc[...] = jnp.zeros(racc.shape, _F32)
        for t in range(1, _NSUB):
            prep_rest(t)
        acc[:, 0:_TM] = down(w0.at[2], h0)
        for t in range(1, _NSUB):
            acc[:, t * _TM:(t + 1) * _TM] = down(w0.at[2], hid0(t))
        pltpu.make_async_copy(wl.at[0:1], wl.at[0:1], sems.at[_S_A]).wait()

    def chunk(j):
        @pl.when(j == 1)
        def _():
            pltpu.make_async_copy(
                wl.at[1:_NL], wl.at[1:_NL], sems.at[_S_B]).wait()

        wg, wu, wd = (wl.at[j, i] for i in range(3))

        wrow = wd[_DM:_D, :].astype(_F32)
        for dd in range(_NV):
            wb[dd] = jnp.broadcast_to(wrow[dd:dd + 1, :], (8, _TF))
        never = flag[0] > 0
        queue = []
        left = {}
        sched = list(_VSCHED)

        def v_finish(t):
            a = t * _TM
            w = _VTILES[t] * 128
            v = acc[_DM:_D, a:a + w] + jnp.sum(racc[:, :, a:a + w], axis=1)
            o_v[_DM:_D, a:a + w] = v.astype(_BF)

            @pl.when(j == _NL - 1)
            def _():
                co(_DM, _D, a, a + w).start()

        def v_phase(markers, frac=1.0):
            n = sched.pop(0)
            units = queue[:n]
            del queue[:n]
            nmk = int(len(markers) * frac)
            gi = 0
            for (t, hf, d0, tt) in units:
                qs = [[] for _ in range(_DG)]
                for rg in range(16):
                    r0 = tt * 128 + rg * 8
                    mk = markers[(gi * nmk) // (n * 16)]
                    gi += 1
                    hs = [jnp.where(never, mk,
                                    hf[r0:r0 + 8, k * 128:(k + 1) * 128])
                          for k in range(_TF // 128)]
                    for i in range(_DG):
                        q = hs[0] * wb[d0 + i, :, 0:128]
                        for k in range(1, _TF // 128):
                            q = q + hs[k] * wb[d0 + i, :, k * 128:(k + 1) * 128]
                        qs[i].append(q)
                c0 = t * _TM + tt * 128
                for i in range(_DG):
                    qt = jnp.concatenate(qs[i], axis=0).T
                    p = racc[d0 + i, :, c0:c0 + 128]
                    for rr in range(16):
                        p = p + qt[rr * 8:(rr + 1) * 8, :]
                    racc[d0 + i, :, c0:c0 + 128] = p
                left[t] -= 1
                if left[t] == 0:
                    v_finish(t)

        for t in range(_NSUB):
            a = t * _TM
            g, gA, gB = proj(wg, t)
            if t > 0:
                v_phase(_vregs(gA) + _vregs(gB))
            hf = _gelu(g) * proj(wu, t)[0]
            h = hf.astype(_BF)
            for tt in range(_VTILES[t]):
                for d0 in range(0, _NV, _DG):
                    queue.append((t, hf, d0, tt))
            left[t] = _VTILES[t] * _NV // _DG
            ds = []
            for grp in _PIECES[t]:
                rows = grp[-1][1]
                pa, pb = grp[0][2], grp[0][3]
                d = down(wd, h[pa - a:pb - a, :], rows)
                ds += _vregs(d)
                v = acc[0:rows, pa:pb] + d
                acc[0:rows, pa:pb] = v
                vb = v.astype(_BF)
                for (r0, r1, _, _) in grp:
                    o_v[r0:r1, pa:pb] = vb[r0:r1, :]

                    @pl.when(j == _NL - 1)
                    def _():
                        co(r0, r1, pa, pb).start()
            v_phase(ds, 1.0 if t < _NSUB - 1 else _VLAST)
        assert not queue and not sched

    def body(j, carry):
        @pl.when(j == 0)
        def _():
            prologue()

        chunk(j)
        return carry

    lax.fori_loop(0, _NL, body, 0)
    pltpu.make_async_copy(o_v, oT_hbm, sems.at[_S_O]).wait()


@jax.jit
def pallas_standalone__geglu_ffn__prompt_kernel(
    x: jax.Array,
    w_gate: jax.Array,
    w_up: jax.Array,
    w_down: jax.Array,
):
    B, S, D = x.shape
    assert B == 1 and (S, D, w_gate.shape[1]) == (_M, _D, _F)
    xT = jnp.swapaxes(x, 1, 2).reshape(_D, _M)
    wdT = w_down.T
    outT = pl.pallas_call(
        _kernel,
        in_specs=[pl.BlockSpec(memory_space=pl.ANY)] * 4,
        out_specs=pl.BlockSpec(memory_space=pl.ANY),
        out_shape=jax.ShapeDtypeStruct((_D, _M), x.dtype),
        scratch_shapes=[
            pltpu.VMEM((_D, _M), _BF),
            pltpu.VMEM((_M // 2, 512), jnp.uint32),
            pltpu.VMEM((_M // 4, 128), jnp.uint32),
            pltpu.VMEM((_M // 2, 128), _F32),
            pltpu.VMEM((3, _D, _TF), _BF),
            pltpu.VMEM((_NL, 3, _D, _TF), _BF),
            pltpu.VMEM((_D, _M), _F32),
            pltpu.VMEM((_D, _M), _BF),
            pltpu.VMEM((2, _M, _TF), _F32),
            pltpu.VMEM((_NV, 8, _TF), _F32),
            pltpu.VMEM((_NV, 8, _VW), _F32),
            pltpu.SMEM((1,), jnp.int32),
            pltpu.SemaphoreType.DMA((_NSEM,)),
        ],
        compiler_params=pltpu.CompilerParams(
            vmem_limit_bytes=100 * 1024 * 1024,
            disable_semaphore_checks=True,
        ),
    )(xT, w_gate, w_up, wdT)
    return jnp.swapaxes(outT.reshape(B, _D, S), 1, 2)
```

```python
import jax
import jax.numpy as jnp
from jax import lax
import jax.experimental.pallas as pl
import jax.experimental.pallas.tpu as pltpu

_NT = (((1,), (1,)), ((), ()))
_BF = jnp.bfloat16
_F32 = jnp.float32

_D, _M, _F = 576, 2048, 4608
_TM = 512
_HM = _TM // 2
_NSUB = _M // _TM
_TF = 512
_NL = _F // _TF - 1

_S_A, _S_B, _S_O, _NSEM = 5, 6, 7, 8

_NV = 16
_DM = _D - _NV
_VTILES = (4, 4, 4, 1)
_VW = 3 * _TM + 128
_DG = 4
_VSCHED = (8, 8, 8, 8, 8, 8, 4)
_VLAST = 0.55

_LAST = (_NSUB - 1) * _TM
_PIECES = [[[(0, _DM, t * _TM, (t + 1) * _TM)]] for t in range(_NSUB - 1)]
_PIECES.append([
    [(0, _DM, _LAST, _LAST + 128)],
    [(0, _D, _LAST + 128, _LAST + 256)],
    [(0, _D, _LAST + 256, _LAST + 384)],
    [(0, _D // 2, _LAST + 384, _M), (_D // 2, _D, _LAST + 384, _M)],
])


def _gelu(g):
    c = 0.7978845608028654
    return 0.5 * g * (1.0 + jnp.tanh(c * (g + 0.044715 * (g * g * g))))


def _pack(v):
    return pltpu.bitcast(v, jnp.uint32)


def _unpack(v):
    return pltpu.bitcast(v, _BF)


def _vregs(v):
    r, c = v.shape
    return [v[i:i + 8, k:k + 128]
            for k in range(0, c, 128) for i in range(0, r, 8)]


def _kernel(xT_hbm, wg_hbm, wu_hbm, wdT_hbm, oT_hbm,
            xT_v, xp, xs, rs, w0, wl, acc, o_v, gu, racc, flag, sems):
    w_hbm = (wg_hbm, wu_hbm, wdT_hbm)
    flag[0] = 0

    def cx(r0, r1, a, b, s):
        return pltpu.make_async_copy(
            xT_hbm.at[r0:r1, a:b], xT_v.at[r0:r1, a:b], sems.at[s])

    def cw(i, r0, r1, s):
        return pltpu.make_async_copy(
            w_hbm[i].at[r0:r1, 0:_TF], w0.at[i, r0:r1, :], sems.at[s])

    def cl(j, i):
        return pltpu.make_async_copy(
            w_hbm[i].at[:, (j + 1) * _TF:(j + 2) * _TF], wl.at[j, i],
            sems.at[_S_A if j == 0 else _S_B])

    def co(r0, r1, a, b):
        return pltpu.make_async_copy(
            o_v.at[r0:r1, a:b], oT_hbm.at[r0:r1, a:b], sems.at[_S_O])

    groups = [
        [cx(0, 128, 0, 512, 0)],
        [cw(0, 0, 128, 1), cw(1, 0, 128, 1)],
        [cx(0, 128, 512, _M, 2)],
        [cx(128, _D, 0, 512, 3), cw(0, 128, _D, 3), cw(1, 128, _D, 3)],
        [cw(2, 0, _D, 4), cx(128, _D, 512, _M, 4)],
    ]
    for grp in groups:
        for c in grp:
            c.start()

    def wait(gi):
        for c in groups[gi]:
            c.wait()

    def prep_k(k, a, b):
        xp[a // 2:b // 2, k * 128:(k + 1) * 128] = _pack(
            xT_v[k * 128:(k + 1) * 128, a:b].T)

    def prep_tail(t):
        a = t * _TM
        b = a + _HM
        s = t * _HM
        A, B = slice(a, a + _HM), slice(b, b + _HM)
        a8 = xT_v[448:512, A].astype(_F32)
        b8 = xT_v[448:512, B].astype(_F32)
        a9 = xT_v[512:576, A].astype(_F32)
        b9 = xT_v[512:576, B].astype(_F32)
        ma = jnp.sum(jnp.abs(a8) + jnp.abs(a9), axis=0, keepdims=True)
        mb = jnp.sum(jnp.abs(b8) + jnp.abs(b9), axis=0, keepdims=True)
        la = jnp.clip(pltpu.bitcast(ma, jnp.int32), 87 << 23, 190 << 23)
        lb = jnp.clip(pltpu.bitcast(mb, jnp.int32), 87 << 23, 190 << 23)
        e = (la - lb + (1 << 22)) >> 23
        r = pltpu.bitcast((127 + e) << 23, _F32)
        rinv = pltpu.bitcast((127 - e) << 23, _F32)
        rb8 = r * b8
        dA = (a8 - rb8).astype(_BF)
        dB = (b9 - rinv * a9).astype(_BF)
        xp[a // 2:b // 2, 384:512] = _pack(
            jnp.concatenate([xT_v[384:448, A], dA], axis=0).T)
        xp[b // 2:(b + _HM) // 2, 384:512] = _pack(
            jnp.concatenate([xT_v[384:448, B], dB], axis=0).T)
        xs[s // 2:(s + _HM) // 2, :] = _pack(
            jnp.concatenate([rb8.astype(_BF), xT_v[512:576, A]], axis=0).T)
        rs[s:s + _HM, :] = jnp.broadcast_to(rinv, (128, _HM)).T

    def prep_rest(t):
        prep_tail(t)
        prep_k(1, t * _TM, (t + 1) * _TM)
        prep_k(2, t * _TM, (t + 1) * _TM)

    def proj(w, t, r0=0):
        a = t * _TM
        b = a + _HM
        s = t * _HM
        pA = jnp.dot(_unpack(xp[a // 2:b // 2, r0:512]), w[r0:512, :],
                     preferred_element_type=_F32)
        wB = jnp.concatenate([w[r0:448, :], w[512:576, :]], axis=0)
        pB = jnp.dot(_unpack(xp[b // 2:(b + _HM) // 2, r0:512]), wB,
                     preferred_element_type=_F32)
        S = jnp.dot(_unpack(xs[s // 2:(s + _HM) // 2, :]), w[448:576, :],
                    preferred_element_type=_F32)
        rinv = jnp.concatenate([rs[s:s + _HM, :]] * (_TF // 128), axis=1)
        return jnp.concatenate([pA + S, pB + S * rinv], axis=0), pA, pB

    def down(wd, h, rows=_D):
        return lax.dot_general(wd[0:rows, :], h, _NT,
                               preferred_element_type=_F32)

    def mm0(i, a, b):
        gu[i, a:b, :] = jnp.dot(_unpack(xp[a // 2:b // 2, 0:128]),
                                w0[i, 0:128, :], preferred_element_type=_F32)

    def hid0(t):
        a = t * _TM
        g = proj(w0.at[0], t, 128)[0] + gu[0, a:a + _TM, :]
        u = proj(w0.at[1], t, 128)[0] + gu[1, a:a + _TM, :]
        return (_gelu(g) * u).astype(_BF)

    def prologue():
        wait(0)
        prep_k(0, 0, 512)
        wait(1)
        mm0(0, 0, 512)
        mm0(1, 0, 256)
        wait(2)
        for j in range(_NL):
            for i in range(3):
                cl(j, i).start()
        for a in range(512, _M, 512):
            prep_k(0, a, a + 512)
        mm0(1, 256, 512)
        for a in (512, 1024):
            mm0(0, a, a + 512)
            mm0(1, a, a + 512)
        mm0(0, 1536, _M)
        wait(3)
        prep_rest(0)
        mm0(1, 1536, _M)
        h0 = hid0(0)
        wait(4)
        racc[...] = jnp.zeros(racc.shape, _F32)
        for t in range(1, _NSUB):
            prep_rest(t)
        acc[:, 0:_TM] = down(w0.at[2], h0)
        for t in range(1, _NSUB):
            acc[:, t * _TM:(t + 1) * _TM] = down(w0.at[2], hid0(t))
        pltpu.make_async_copy(wl.at[0:1], wl.at[0:1], sems.at[_S_A]).wait()

    def chunk(j):
        @pl.when(j == 1)
        def _():
            pltpu.make_async_copy(
                wl.at[1:_NL], wl.at[1:_NL], sems.at[_S_B]).wait()

        wg, wu, wd = (wl.at[j, i] for i in range(3))

        wrow = wd[_DM:_D, :].astype(_F32)
        wrep = [jnp.concatenate(
            [jnp.broadcast_to(wrow[dd:dd + 1, :], (8, _TF))
             for dd in range(d0, d0 + _DG)], axis=0)
            for d0 in range(0, _NV, _DG)]
        never = flag[0] > 0
        queue = []
        left = {}
        sched = list(_VSCHED)

        def v_finish(t):
            a = t * _TM
            w = _VTILES[t] * 128
            v = acc[_DM:_D, a:a + w] + jnp.sum(racc[:, :, a:a + w], axis=1)
            o_v[_DM:_D, a:a + w] = v.astype(_BF)

            @pl.when(j == _NL - 1)
            def _():
                co(_DM, _D, a, a + w).start()

        def v_phase(markers, frac=1.0):
            n = sched.pop(0)
            units = queue[:n]
            del queue[:n]
            nmk = int(len(markers) * frac)
            gi = 0
            for (t, hf, d0, tt) in units:
                qs = []
                for rg in range(16):
                    r0 = tt * 128 + rg * 8
                    mk = markers[(gi * nmk) // (n * 16)]
                    gi += 1
                    hs = jnp.where(
                        never, jnp.concatenate([mk] * (_TF // 128), axis=1),
                        hf[r0:r0 + 8, :])
                    p = jnp.concatenate([hs] * _DG, axis=0) * wrep[d0 // _DG]
                    q = p[:, 0:128]
                    for k in range(1, _TF // 128):
                        q = q + p[:, k * 128:(k + 1) * 128]
                    qs.append(q)
                c0 = t * _TM + tt * 128
                ps = []
                for i in range(_DG):
                    qt = jnp.concatenate(
                        [q[i * 8:(i + 1) * 8, :] for q in qs], axis=0).T
                    ps.append(jnp.sum(qt.reshape(16, 8, 128), axis=0))
                racc[d0:d0 + _DG, :, c0:c0 + 128] += jnp.stack(ps, axis=0)
                left[t] -= 1
                if left[t] == 0:
                    v_finish(t)

        for t in range(_NSUB):
            a = t * _TM
            g, gA, gB = proj(wg, t)
            if t > 0:
                v_phase(_vregs(gA) + _vregs(gB))
            hf = _gelu(g) * proj(wu, t)[0]
            h = hf.astype(_BF)
            for tt in range(_VTILES[t]):
                for d0 in range(0, _NV, _DG):
                    queue.append((t, hf, d0, tt))
            left[t] = _VTILES[t] * _NV // _DG
            ds = []
            for grp in _PIECES[t]:
                rows = grp[-1][1]
                pa, pb = grp[0][2], grp[0][3]
                d = down(wd, h[pa - a:pb - a, :], rows)
                ds += _vregs(d)
                v = acc[0:rows, pa:pb] + d
                acc[0:rows, pa:pb] = v
                vb = v.astype(_BF)
                for (r0, r1, _, _) in grp:
                    o_v[r0:r1, pa:pb] = vb[r0:r1, :]

                    @pl.when(j == _NL - 1)
                    def _():
                        co(r0, r1, pa, pb).start()
            v_phase(ds, 1.0 if t < _NSUB - 1 else _VLAST)
        assert not queue and not sched

    def body(j, carry):
        @pl.when(j == 0)
        def _():
            prologue()

        chunk(j)
        return carry

    lax.fori_loop(0, _NL, body, 0)
    pltpu.make_async_copy(o_v, oT_hbm, sems.at[_S_O]).wait()


@jax.jit
def pallas_standalone__geglu_ffn__prompt_kernel(
    x: jax.Array,
    w_gate: jax.Array,
    w_up: jax.Array,
    w_down: jax.Array,
):
    B, S, D = x.shape
    assert B == 1 and (S, D, w_gate.shape[1]) == (_M, _D, _F)
    xT = jnp.swapaxes(x, 1, 2).reshape(_D, _M)
    wdT = w_down.T
    outT = pl.pallas_call(
        _kernel,
        in_specs=[pl.BlockSpec(memory_space=pl.ANY)] * 4,
        out_specs=pl.BlockSpec(memory_space=pl.ANY),
        out_shape=jax.ShapeDtypeStruct((_D, _M), x.dtype),
        scratch_shapes=[
            pltpu.VMEM((_D, _M), _BF),
            pltpu.VMEM((_M // 2, 512), jnp.uint32),
            pltpu.VMEM((_M // 4, 128), jnp.uint32),
            pltpu.VMEM((_M // 2, 128), _F32),
            pltpu.VMEM((3, _D, _TF), _BF),
            pltpu.VMEM((_NL, 3, _D, _TF), _BF),
            pltpu.VMEM((_D, _M), _F32),
            pltpu.VMEM((_D, _M), _BF),
            pltpu.VMEM((2, _M, _TF), _F32),
            pltpu.VMEM((_NV, 8, _VW), _F32),
            pltpu.SMEM((1,), jnp.int32),
            pltpu.SemaphoreType.DMA((_NSEM,)),
        ],
        compiler_params=pltpu.CompilerParams(
            vmem_limit_bytes=100 * 1024 * 1024,
            disable_semaphore_checks=True,
        ),
    )(xT, w_gate, w_up, wdT)
    return jnp.swapaxes(outT.reshape(B, _D, S), 1, 2)
```

```python
import jax
import jax.numpy as jnp
from jax import lax
import jax.experimental.pallas as pl
import jax.experimental.pallas.tpu as pltpu

_NT = (((1,), (1,)), ((), ()))
_BF = jnp.bfloat16
_F32 = jnp.float32

_D, _M, _F = 576, 2048, 4608
_TM = 512
_HM = _TM // 2
_NSUB = _M // _TM
_TF = 512
_NL = _F // _TF - 1

_S_A, _S_B, _S_O, _NSEM = 5, 6, 7, 8

_NV = 16
_DM = _D - _NV
_VTILES = (4, 4, 4, 2)
_VW = 3 * _TM + 256
_DG = 4
_VSCHED = (8, 8, 8, 8, 8, 8, 8)
_VLAST = 0.85

_LAST = (_NSUB - 1) * _TM
_PIECES = [[[(0, _DM, t * _TM, (t + 1) * _TM)]] for t in range(_NSUB - 1)]
_PIECES.append([
    [(0, _DM, _LAST, _LAST + 256)],
    [(0, _D, _LAST + 256, _LAST + 384)],
    [(0, _D // 2, _LAST + 384, _M), (_D // 2, _D, _LAST + 384, _M)],
])


def _gelu(g):
    c = 0.7978845608028654
    return 0.5 * g * (1.0 + jnp.tanh(c * (g + 0.044715 * (g * g * g))))


def _pack(v):
    return pltpu.bitcast(v, jnp.uint32)


def _unpack(v):
    return pltpu.bitcast(v, _BF)


def _vregs(v):
    r, c = v.shape
    return [v[i:i + 8, k:k + 128]
            for k in range(0, c, 128) for i in range(0, r, 8)]


def _kernel(xT_hbm, wg_hbm, wu_hbm, wdT_hbm, oT_hbm,
            xT_v, xp, xs, rs, w0, wl, acc, o_v, gu, racc, flag, sems):
    w_hbm = (wg_hbm, wu_hbm, wdT_hbm)
    flag[0] = 0

    def cx(r0, r1, a, b, s):
        return pltpu.make_async_copy(
            xT_hbm.at[r0:r1, a:b], xT_v.at[r0:r1, a:b], sems.at[s])

    def cw(i, r0, r1, s):
        return pltpu.make_async_copy(
            w_hbm[i].at[r0:r1, 0:_TF], w0.at[i, r0:r1, :], sems.at[s])

    def cl(j, i):
        return pltpu.make_async_copy(
            w_hbm[i].at[:, (j + 1) * _TF:(j + 2) * _TF], wl.at[j, i],
            sems.at[_S_A if j == 0 else _S_B])

    def co(r0, r1, a, b):
        return pltpu.make_async_copy(
            o_v.at[r0:r1, a:b], oT_hbm.at[r0:r1, a:b], sems.at[_S_O])

    groups = [
        [cx(0, 128, 0, 512, 0)],
        [cw(0, 0, 128, 1), cw(1, 0, 128, 1)],
        [cx(0, 128, 512, _M, 2)],
        [cx(128, _D, 0, 512, 3), cw(0, 128, _D, 3), cw(1, 128, _D, 3)],
        [cw(2, 0, _D, 4), cx(128, _D, 512, _M, 4)],
    ]
    for grp in groups:
        for c in grp:
            c.start()

    def wait(gi):
        for c in groups[gi]:
            c.wait()

    def prep_k(k, a, b):
        xp[a // 2:b // 2, k * 128:(k + 1) * 128] = _pack(
            xT_v[k * 128:(k + 1) * 128, a:b].T)

    def prep_tail(t):
        a = t * _TM
        b = a + _HM
        s = t * _HM
        A, B = slice(a, a + _HM), slice(b, b + _HM)
        a8 = xT_v[448:512, A].astype(_F32)
        b8 = xT_v[448:512, B].astype(_F32)
        a9 = xT_v[512:576, A].astype(_F32)
        b9 = xT_v[512:576, B].astype(_F32)
        ma = jnp.sum(jnp.abs(a8) + jnp.abs(a9), axis=0, keepdims=True)
        mb = jnp.sum(jnp.abs(b8) + jnp.abs(b9), axis=0, keepdims=True)
        la = jnp.clip(pltpu.bitcast(ma, jnp.int32), 87 << 23, 190 << 23)
        lb = jnp.clip(pltpu.bitcast(mb, jnp.int32), 87 << 23, 190 << 23)
        e = (la - lb + (1 << 22)) >> 23
        r = pltpu.bitcast((127 + e) << 23, _F32)
        rinv = pltpu.bitcast((127 - e) << 23, _F32)
        rb8 = r * b8
        dA = (a8 - rb8).astype(_BF)
        dB = (b9 - rinv * a9).astype(_BF)
        xp[a // 2:b // 2, 384:512] = _pack(
            jnp.concatenate([xT_v[384:448, A], dA], axis=0).T)
        xp[b // 2:(b + _HM) // 2, 384:512] = _pack(
            jnp.concatenate([xT_v[384:448, B], dB], axis=0).T)
        xs[s // 2:(s + _HM) // 2, :] = _pack(
            jnp.concatenate([rb8.astype(_BF), xT_v[512:576, A]], axis=0).T)
        rs[s:s + _HM, :] = jnp.broadcast_to(rinv, (128, _HM)).T

    def prep_rest(t):
        prep_tail(t)
        prep_k(1, t * _TM, (t + 1) * _TM)
        prep_k(2, t * _TM, (t + 1) * _TM)

    def proj(w, t, r0=0):
        a = t * _TM
        b = a + _HM
        s = t * _HM
        pA = jnp.dot(_unpack(xp[a // 2:b // 2, r0:512]), w[r0:512, :],
                     preferred_element_type=_F32)
        wB = jnp.concatenate([w[r0:448, :], w[512:576, :]], axis=0)
        pB = jnp.dot(_unpack(xp[b // 2:(b + _HM) // 2, r0:512]), wB,
                     preferred_element_type=_F32)
        S = jnp.dot(_unpack(xs[s // 2:(s + _HM) // 2, :]), w[448:576, :],
                    preferred_element_type=_F32)
        rinv = jnp.concatenate([rs[s:s + _HM, :]] * (_TF // 128), axis=1)
        return jnp.concatenate([pA + S, pB + S * rinv], axis=0), pA, pB

    def down(wd, h, rows=_D):
        return lax.dot_general(wd[0:rows, :], h, _NT,
                               preferred_element_type=_F32)

    def mm0(i, a, b):
        gu[i, a:b, :] = jnp.dot(_unpack(xp[a // 2:b // 2, 0:128]),
                                w0[i, 0:128, :], preferred_element_type=_F32)

    def hid0(t):
        a = t * _TM
        g = proj(w0.at[0], t, 128)[0] + gu[0, a:a + _TM, :]
        u = proj(w0.at[1], t, 128)[0] + gu[1, a:a + _TM, :]
        return (_gelu(g) * u).astype(_BF)

    def prologue():
        racc[...] = jnp.zeros(racc.shape, _F32)
        wait(0)
        prep_k(0, 0, 512)
        wait(1)
        mm0(0, 0, 512)
        mm0(1, 0, 256)
        wait(2)
        for j in range(_NL):
            for i in range(3):
                cl(j, i).start()
        for a in range(512, _M, 512):
            prep_k(0, a, a + 512)
        mm0(1, 256, 512)
        for a in (512, 1024):
            mm0(0, a, a + 512)
            mm0(1, a, a + 512)
        mm0(0, 1536, _M)
        wait(3)
        prep_rest(0)
        mm0(1, 1536, _M)
        h0 = hid0(0)
        wait(4)
        for t in range(1, _NSUB):
            prep_rest(t)
        acc[:, 0:_TM] = down(w0.at[2], h0)
        for t in range(1, _NSUB):
            acc[:, t * _TM:(t + 1) * _TM] = down(w0.at[2], hid0(t))
        pltpu.make_async_copy(wl.at[0:1], wl.at[0:1], sems.at[_S_A]).wait()

    def chunk(j):
        @pl.when(j == 1)
        def _():
            pltpu.make_async_copy(
                wl.at[1:_NL], wl.at[1:_NL], sems.at[_S_B]).wait()

        wg, wu, wd = (wl.at[j, i] for i in range(3))

        wrow = wd[_DM:_D, :].astype(_F32)
        wrep = [jnp.concatenate(
            [jnp.broadcast_to(wrow[dd:dd + 1, :], (8, _TF))
             for dd in range(d0, d0 + _DG)], axis=0)
            for d0 in range(0, _NV, _DG)]
        never = flag[0] > 0
        queue = []
        left = {}
        sched = list(_VSCHED)

        def v_finish(t):
            a = t * _TM
            w = _VTILES[t] * 128
            v = acc[_DM:_D, a:a + w] + jnp.sum(racc[:, :, a:a + w], axis=1)
            o_v[_DM:_D, a:a + w] = v.astype(_BF)

            @pl.when(j == _NL - 1)
            def _():
                co(_DM, _D, a, a + w).start()

        def v_phase(markers, frac=1.0):
            n = sched.pop(0)
            units = queue[:n]
            del queue[:n]
            nmk = int(len(markers) * frac)
            gi = 0
            for (t, hf, d0, tt) in units:
                qs = []
                for rg in range(16):
                    r0 = tt * 128 + rg * 8
                    mk = markers[(gi * nmk) // (n * 16)]
                    gi += 1
                    hs = jnp.where(
                        never, jnp.concatenate([mk] * (_TF // 128), axis=1),
                        hf[r0:r0 + 8, :])
                    p = jnp.concatenate([hs] * _DG, axis=0) * wrep[d0 // _DG]
                    q = p[:, 0:128]
                    for k in range(1, _TF // 128):
                        q = q + p[:, k * 128:(k + 1) * 128]
                    qs.append(q)
                c0 = t * _TM + tt * 128
                ps = []
                for i in range(_DG):
                    qt = jnp.concatenate(
                        [q[i * 8:(i + 1) * 8, :] for q in qs], axis=0).T
                    ps.append(jnp.sum(qt.reshape(16, 8, 128), axis=0))
                racc[d0:d0 + _DG, :, c0:c0 + 128] += jnp.stack(ps, axis=0)
                left[t] -= 1
                if left[t] == 0:
                    v_finish(t)

        for t in range(_NSUB):
            a = t * _TM
            g, gA, gB = proj(wg, t)
            if t > 0:
                v_phase(_vregs(gA) + _vregs(gB))
            hf = _gelu(g) * proj(wu, t)[0]
            h = hf.astype(_BF)
            for tt in range(_VTILES[t]):
                for d0 in range(0, _NV, _DG):
                    queue.append((t, hf, d0, tt))
            left[t] = _VTILES[t] * _NV // _DG
            ds = []
            for grp in _PIECES[t]:
                rows = grp[-1][1]
                pa, pb = grp[0][2], grp[0][3]
                d = down(wd, h[pa - a:pb - a, :], rows)
                ds += _vregs(d)
                v = acc[0:rows, pa:pb] + d
                acc[0:rows, pa:pb] = v
                vb = v.astype(_BF)
                for (r0, r1, _, _) in grp:
                    o_v[r0:r1, pa:pb] = vb[r0:r1, :]

                    @pl.when(j == _NL - 1)
                    def _():
                        co(r0, r1, pa, pb).start()
            v_phase(ds, 1.0 if t < _NSUB - 1 else _VLAST)
        assert not queue and not sched

    def body(j, carry):
        @pl.when(j == 0)
        def _():
            prologue()

        chunk(j)
        return carry

    lax.fori_loop(0, _NL, body, 0)
    pltpu.make_async_copy(o_v, oT_hbm, sems.at[_S_O]).wait()


@jax.jit
def pallas_standalone__geglu_ffn__prompt_kernel(
    x: jax.Array,
    w_gate: jax.Array,
    w_up: jax.Array,
    w_down: jax.Array,
):
    B, S, D = x.shape
    assert B == 1 and (S, D, w_gate.shape[1]) == (_M, _D, _F)
    xT = jnp.swapaxes(x, 1, 2).reshape(_D, _M)
    wdT = w_down.T
    outT = pl.pallas_call(
        _kernel,
        in_specs=[pl.BlockSpec(memory_space=pl.ANY)] * 4,
        out_specs=pl.BlockSpec(memory_space=pl.ANY),
        out_shape=jax.ShapeDtypeStruct((_D, _M), x.dtype),
        scratch_shapes=[
            pltpu.VMEM((_D, _M), _BF),
            pltpu.VMEM((_M // 2, 512), jnp.uint32),
            pltpu.VMEM((_M // 4, 128), jnp.uint32),
            pltpu.VMEM((_M // 2, 128), _F32),
            pltpu.VMEM((3, _D, _TF), _BF),
            pltpu.VMEM((_NL, 3, _D, _TF), _BF),
            pltpu.VMEM((_D, _M), _F32),
            pltpu.VMEM((_D, _M), _BF),
            pltpu.VMEM((2, _M, _TF), _F32),
            pltpu.VMEM((_NV, 8, _VW), _F32),
            pltpu.SMEM((1,), jnp.int32),
            pltpu.SemaphoreType.DMA((_NSEM,)),
        ],
        compiler_params=pltpu.CompilerParams(
            vmem_limit_bytes=100 * 1024 * 1024,
            disable_semaphore_checks=True,
        ),
    )(xT, w_gate, w_up, wdT)
    return jnp.swapaxes(outT.reshape(B, _D, S), 1, 2)
```
